```python
import os as _os
_os.environ.setdefault("JAX_PLATFORMS", "cpu")
import jax
import jax.numpy as jnp

def _softmax(x, axis=-1):
    return jax.nn.softmax(x, axis=axis)
def _gelu(x):
    return jax.nn.gelu(x, approximate=True)
def _silu(x):
    return jax.nn.silu(x)
def _sigmoid(x):
    return jax.nn.sigmoid(x)
def _layernorm(x, axis=-1, eps=1e-5):
    m = jnp.mean(x, axis=axis, keepdims=True)
    v = jnp.var(x, axis=axis, keepdims=True)
    return (x - m) / jnp.sqrt(v + eps)
def _scatter_add(tgt, idx, src, axis=0):
    return tgt.at[idx].add(src)
def _segment_sum(src, seg, n):
    return jax.ops.segment_sum(src, seg, n)
class _Rng:
    def __init__(self, key):
        self._k = key
    def _next(self):
        self._k, sub = jax.random.split(self._k)
        return sub
    def normal(self, shape):
        return jax.random.normal(self._next(), shape, dtype=jnp.bfloat16)
    def randint(self, lo, hi, shape):
        return jax.random.randint(self._next(), shape, lo, hi, dtype=jnp.int32)
    def uniform(self, shape, lo=0.0, hi=1.0):
        return jax.random.uniform(self._next(), shape, jnp.bfloat16, lo, hi)
    def permutation(self, n):
        return jax.random.permutation(self._next(), n)


kernel_name = 'sequential_preLN__sliding_block__dense_activation_relu__prompt'

def setup_inputs():
    _rng = _Rng(jax.random.key(int.from_bytes(__import__("os").urandom(4), "little")))
    _w = (lambda a: (lambda t: t.astype(jnp.bfloat16) if jnp.issubdtype(t.dtype, jnp.floating) else t)(jnp.asarray(a)))
    def _A_setup():
        B, S, D = 1, 2048, 640
        return {
            "x": _w((lambda *s: _rng.normal(s) * 0.05)(B, S, D)),
            "wqkv": _w((lambda *s: _rng.normal(s) * 0.05)(D, 3 * D)),
            "wo": _w((lambda *s: _rng.normal(s) * 0.05)(D, D)),
        }
    _A_in = _A_setup()

    def _B_setup():
        B, S, D, Dff = 1, 2048, 640, 1536
        return {
            "x": _w((lambda *s: _rng.normal(s) * 0.05)(B, S, D)),
            "w1": _w((lambda *s: _rng.normal(s) * 0.05)(D, Dff)),
            "w2": _w((lambda *s: _rng.normal(s) * 0.05)(Dff, D)),
        }
    _B_in = _B_setup()

    return {
        "A_x": _A_in["x"],
        "A_wqkv": _A_in["wqkv"],
        "A_wo": _A_in["wo"],
        "B_x": _B_in["x"],
        "B_w1": _B_in["w1"],
        "B_w2": _B_in["w2"],
    }

def reference(A_x, A_wqkv, A_wo, B_x, B_w1, B_w2):
    def _A_ref(x, wqkv, wo):
        B, S, D = x.shape
        H = 32; Dh = D // H; W = 256
        qkv = (lambda x, *d: x.transpose(*d))((x @ wqkv).reshape(B, S, 3, H, Dh), 2, 0, 3, 1, 4)
        q, k, v = qkv[0], qkv[1], qkv[2]
        scores = jnp.einsum("bhqd,bhkd->bhqk", q, k) * (Dh ** -0.5)
        idx = jnp.arange(S)
        mask = (idx[:, None] - idx[None, :] >= 0) & (idx[:, None] - idx[None, :] < W)
        scores = jnp.where(mask[None, None], scores, -1e9)
        p = _softmax(scores, axis=-1)
        o = jnp.einsum("bhqk,bhkd->bhqd", p, v)
        return (lambda x, *d: x.transpose(*d))(o, 0, 2, 1, 3).reshape(B, S, D) @ wo

    def _B_ref(x, w1, w2):
        h = jnp.einsum("bsd,df->bsf", x, w1)
        zero = jnp.zeros_like(h)
        h = jnp.maximum(h, zero)
        return jnp.einsum("bsf,fd->bsd", h, w2)

    x = A_x
    h = x + _A_ref(_layernorm(x, axis=-1), A_wqkv, A_wo)
    h2 = h + _B_ref(_layernorm(h, axis=-1), B_w1, B_w2)
    return h2
```

```python
import functools
import math
import jax
import jax.numpy as jnp
from jax import lax
from jax.experimental import pallas as pl
from jax.experimental.pallas import tpu as pltpu

S, D, H, DH, W, DFF = 2048, 640, 32, 20, 256, 1536
NQUAD = 8
EPS = 1e-5
QSCALE = (DH ** -0.5) * math.log2(math.e)
NEG = -1e30
F32 = jnp.float32
BF16 = jnp.bfloat16
U32 = jnp.uint32
ONES = 0x3F803F80
NT = (((1,), (1,)), ((), ()))
TQ = 256
NSB = TQ // 128
NB = S // TQ
SCOPES = False


def _ln(x):
    mu = jnp.mean(x, axis=-1, keepdims=True)
    xc = x - mu
    var = jnp.mean(xc * xc, axis=-1, keepdims=True)
    return xc * lax.rsqrt(var + EPS)


def _pack(x_bf16):
    return pltpu.bitcast(x_bf16, U32)


def _unpack(x_u32):
    return pltpu.bitcast(x_u32, BF16)


def _ipack(x):
    n, L = x.shape[0] // 16, x.shape[1]
    x3 = x.reshape(n, 16, L)
    return pltpu.pack_elementwise(
        [x3[:, 0:8, :].reshape(8 * n, L), x3[:, 8:16, :].reshape(8 * n, L)], packed_dtype=BF16)


def _lane_in(lane, lo, n):
    lo = lo % 128
    hi = lo + n
    if hi <= 128:
        return (lane >= lo) & (lane < hi)
    return (lane >= lo) | (lane < hi - 128)


def _quad_src(xp, m, lane):
    lo = 80 * m
    hi = lo + 80
    t0, t1 = lo // 128, (hi - 1) // 128
    a = xp[:, 128 * t0:128 * t0 + 128]
    if t0 == t1:
        return a
    return jnp.where(lane >= 64, a, xp[:, 128 * t1:128 * t1 + 128])


_ONE_ROW = {0: 20, 4: 0, 8: 28, 12: 8}


def _dot(a, b):
    return jnp.dot(a, b, preferred_element_type=F32)


def _rows(t, n):
    if isinstance(t, int):
        return t * n
    return pl.multiple_of(t * n, n)


class _NoScope:
    def __init__(self, name):
        pass

    def __enter__(self):
        return self

    def __exit__(self, *a):
        return False


def make_kernel(LA, FR, F1C, F2C, skew, PVD, mode, lead, extra, stS, stP, pre, lnpos, tail, edge):
    nodma = extra is not None
    scope = _NoScope

    def kernel(x_hbm, wqkv_hbm, wo_hbm, w1_hbm, w2_hbm, out_hbm,
               x_v, out_v, wqkv_ref, wo_ref, w1_ref, w2_ref, wvt_ref, k_ref, vt_ref, q_ref,
               os_ref, h1_ref, hn_ref, s_ref, p_ref, wsem, xsem, osem):

        def cp_qkv(j):
            return pltpu.make_async_copy(wqkv_hbm.at[:, pl.ds(j * D, D)], wqkv_ref.at[:, pl.ds(j * D, D)], wsem.at[j])
        cp_wo = pltpu.make_async_copy(wo_hbm, wo_ref, wsem.at[3])
        cp_w1 = pltpu.make_async_copy(w1_hbm, w1_ref, wsem.at[4])
        cp_w2 = pltpu.make_async_copy(w2_hbm, w2_ref, wsem.at[5])

        def cp_x(t):
            r = pl.ds(_rows(t, TQ), TQ)
            return pltpu.make_async_copy(x_hbm.at[r], x_v.at[r], xsem.at[t])

        def cp_out(t, r):
            rr = pl.ds(_rows(t, TQ) + FR * r, FR)
            return pltpu.make_async_copy(out_v.at[rr], out_hbm.at[rr], osem.at[t * (TQ // FR) + r])

        def stage_a(t, first=False, wait=True):
            st = {}

            def ln1():
                if (not nodma or first) and wait:
                    cp_x(t).wait()
                xnf = _ln(x_v[pl.ds(_rows(t, TQ), TQ), :].astype(F32))
                st["xn"] = xnf.astype(BF16)
                st["xni"] = _unpack(_ipack(xnf))

            def proj_k():
                if first:
                    cp_qkv(1).wait()
                kp = _pack(_dot(st["xn"], wqkv_ref[:, D:2 * D]).astype(BF16))
                lane_h = lax.broadcasted_iota(jnp.int32, (TQ // 2, 128), 1)
                for m in range(NQUAD):
                    k_ref[m, pl.ds(_rows(t, TQ // 2), TQ // 2), :] = _quad_src(kp, m, lane_h)

            def proj_q():
                if first:
                    cp_qkv(0).wait()
                qp = _pack((_dot(st["xn"], wqkv_ref[:, 0:D]) * QSCALE).astype(BF16))
                lane_h = lax.broadcasted_iota(jnp.int32, (TQ // 2, 128), 1)
                for m in range(NQUAD):
                    q_ref[t % 2, m] = _quad_src(qp, m, lane_h)

            def proj_v():
                if first:
                    cp_qkv(2).wait()
                    wp = _pack(wqkv_ref[:, 2 * D:3 * D].T)
                    ev = pltpu.unpack_elementwise(wp, index=0, packed_dtype=BF16, unpacked_dtype=F32)
                    od = pltpu.unpack_elementwise(wp, index=1, packed_dtype=BF16, unpacked_dtype=F32)
                    wd = jnp.concatenate([ev.reshape(D // 16, 8, D), od.reshape(D // 16, 8, D)], axis=1)
                    wvt_ref[...] = wd.reshape(D, D).astype(BF16)
                vt = lax.dot_general(wvt_ref[...], st["xni"], NT, preferred_element_type=F32)
                vtp = _ipack(vt)
                sub16 = lax.broadcasted_iota(jnp.int32, (16, 128), 0)
                for sb in range(NSB):
                    for h in range(H):
                        ws = 16 * ((20 * h) // 16)
                        r1 = _ONE_ROW[20 * h - ws]
                        win = vtp[ws // 2:ws // 2 + 16, 128 * sb:128 * sb + 128]
                        vt_ref[t * NSB + sb, 16 * h:16 * h + 16, :] = jnp.where(
                            sub16 == r1 // 2, jnp.uint32(ONES), win)
            w = TQ * 25
            return dict(ln=(0, ln1), k=(w, proj_k), q=(w, proj_q), v=(w, proj_v))

        def attention(t):
            clipped = isinstance(t, int) and t == 0
            lane64 = lax.broadcasted_iota(jnp.int32, (64, 128), 1)
            lane16 = lax.broadcasted_iota(jnp.int32, (16, 128), 1)
            r32 = lax.broadcasted_iota(jnp.int32, (32, 128), 0)
            c32 = lax.broadcasted_iota(jnp.int32, (32, 128), 1) % 32
            tri = r32 > c32
            sub8 = lax.broadcasted_iota(jnp.int32, (8, 128), 0)
            odd = (lane16 & 32) != 0
            hi = (lane16 & 64) != 0

            def sel(msk, tv, fv):
                if tv is None and fv is None:
                    return None
                z = jnp.zeros((16, 128), U32)
                return jnp.where(msk, tv if tv is not None else z, fv if fv is not None else z)

            def stage_q(sb, m):
                qt = q_ref[t % 2, m, 64 * sb:64 * sb + 64, :]
                return [jnp.where(_lane_in(lane64, 80 * m + 20 * k, 20), qt, jnp.uint32(0)) for k in range(4)]

            def stage_s(sb, m, g, qm):
                rhs = _unpack(jnp.concatenate([qm[(g - p) % 4][16 * g:16 * g + 16] for p in range(4)], axis=0))
                if clipped:
                    n = 128 * sb + 32 * (g + 1)
                    s = lax.dot_general(_unpack(k_ref[m, 0:n // 2, :]), rhs, NT, preferred_element_type=F32)
                    last = jnp.where(tri, NEG, s[n - 32:n])
                    mm = jnp.concatenate([s[0:n - 32], last], axis=0) if n > 32 else last
                else:
                    r0 = (t * NSB + sb - 2) * 64 + 16 * g
                    if not isinstance(r0, int):
                        r0 = pl.multiple_of(r0, 16)
                    s = lax.dot_general(_unpack(k_ref[m, pl.ds(r0, 144), :]), rhs, NT, preferred_element_type=F32)
                    top = jnp.where(tri, s[0:32], s[256:288])
                    mm = jnp.concatenate([top, s[32:256]], axis=0)
                return mm, jnp.max(mm, axis=0, keepdims=True)

            def stage_e(mm, mx):
                e = jnp.exp2(mm - mx)
                if clipped:
                    return _ipack(e)
                et = e[0:32]
                return _ipack(jnp.concatenate(
                    [jnp.where(tri, et, 0.0), e[32:256], jnp.where(tri, 0.0, et)], axis=0))

            def stage_pv(sb, m, P, par):
                if clipped:
                    nR, off, vb0 = 4 * (sb + 1), [0, 0, 0, 0], 0
                else:
                    nR, off, vb0 = 12, [0, 1, 2, 3], t * NSB + sb - 2
                blocks = {par: [], par + 2: []}
                for R in range(nR):
                    A = []
                    for g in range(4):
                        j = R - off[g]
                        A.append(P[g][16 * j:16 * j + 16] if 0 <= j < P[g].shape[0] // 16 else None)
                    b0 = sel(odd, A[(par + 1) % 4], A[par])
                    b2 = sel(odd, A[(par + 3) % 4], A[par + 2])
                    for k, o in ((par, sel(hi, b2, b0)), (par + 2, sel(hi, b0, b2))):
                        blocks[k].append(o if o is not None else jnp.zeros((16, 128), U32))
                res = {}
                for k in (par, par + 2):
                    h = 4 * m + k
                    ws = 16 * ((20 * h) // 16)
                    r1 = _ONE_ROW[20 * h - ws]
                    pk = _unpack(jnp.concatenate(blocks[k], axis=0))
                    vws = [vt_ref[vb0 + i, 16 * h:16 * h + 16, :] for i in range(nR // 4)]
                    vwin = jnp.concatenate(vws, axis=1) if len(vws) > 1 else vws[0]
                    o = _dot(_unpack(vwin), pk)
                    a = 8 * ((20 * h) // 8) - ws
                    o = o[a:a + 24] * (1.0 / o[r1:r1 + 1])
                    if k:
                        o = pltpu.roll(o, 32 * k, 1)
                    res[k] = o
                return res

            items = [(sb, m) for sb in range(NSB) for m in range(NQUAD)]
            units = [(it, g) for it in items for g in range(4)]
            n = len(units)
            Sv, Pv, Q, O, rows = {}, {}, {}, {}, {}
            pv_at = {}
            for qi in range(len(items)):
                pv_at.setdefault(4 * qi + 3 + PVD[0], []).append((qi, 0))
                pv_at.setdefault(4 * qi + 3 + PVD[1], []).append((qi, 1))
            for u in range(-LA, n + max(PVD)):
                wgt = 0
                us = u + LA
                if 0 <= us < n:
                    it, g = units[us]
                    if g == 0:
                        Q[it] = stage_q(*it)
                    mm_, mx_ = stage_s(*it, g, Q[it])
                    if stS:
                        s_ref[us, 0:mm_.shape[0], :] = mm_
                        Sv[us] = (mm_.shape[0], mx_)
                    else:
                        Sv[us] = (mm_, mx_)
                    wgt += 1
                if 0 <= u < n:
                    mm_, mx_ = Sv.pop(u)
                    if stS:
                        mm_ = s_ref[u, 0:mm_, :]
                    pp = stage_e(mm_, mx_)
                    if stP:
                        p_ref[u, 0:pp.shape[0], :] = pp
                        Pv[u] = p_ref.at[u, 0:pp.shape[0], :]
                    else:
                        Pv[u] = pp
                    wgt += 1
                for qi, par in pv_at.get(u, []):
                    sb, m = items[qi]
                    O.setdefault(qi, {}).update(stage_pv(sb, m, [Pv[4 * qi + g] for g in range(4)], par))
                    if len(O[qi]) == 4:
                        o24 = O.pop(qi)
                        rr = []
                        for pr in range(2):
                            ev, od = o24[2 * pr], o24[2 * pr + 1]
                            rr += [ev[0:16], jnp.where(sub8 < 4, ev[16:24], od[0:8]), od[8:24]]
                        rows[(sb, m)] = rr
                        if m == NQUAD - 1:
                            ot = jnp.concatenate(sum([rows.pop((sb, mm_)) for mm_ in range(NQUAD)], []), axis=0)
                            os_ref[128 * sb:128 * sb + 128, :] = ot.T.astype(BF16)
                yield

        NSTEPS = NSB * NQUAD * 4 + LA + max(PVD)

        def oproj(t):
            h1_ref[...] = x_v[pl.ds(_rows(t, TQ), TQ), :].astype(F32) + _dot(os_ref[...], wo_ref[...])

        def ln2():
            hn_ref[...] = _ln(h1_ref[...]).astype(BF16)

        def ffn(t, start=True):
            thunks = []
            f = {}
            for r in range(TQ // FR):
                rs = slice(FR * r, FR * r + FR)
                for c in range(DFF // F1C):
                    def t1(r=r, rs=rs, c=c):
                        f[(r, c)] = jnp.maximum(_dot(hn_ref[rs, :], w1_ref[:, F1C * c:F1C * c + F1C]), 0.0).astype(BF16)
                    thunks.append((FR * 5 * (F1C // 128), t1))
                for c0 in range(0, D, F2C):
                    c1 = min(D, c0 + F2C)

                    def t2(r=r, rs=rs, c0=c0, c1=c1):
                        acc = h1_ref[rs, c0:c1]
                        for c in range(DFF // F1C):
                            acc = acc + _dot(f[(r, c)], w2_ref[F1C * c:F1C * c + F1C, c0:c1])
                        out_v[pl.ds(_rows(t, TQ) + FR * r, FR), c0:c1] = acc.astype(BF16)
                        if c1 == D and not nodma and start:
                            cp_out(t, r).start()
                    thunks.append((FR * 12 * ((c1 - c0) // 128), t2))
            return thunks

        def run_mixed(gen, thunks):
            total = sum(w for w, _ in thunks)
            done = 0
            ti = 0
            for i, _ in enumerate(gen):
                while ti < len(thunks) and (done + thunks[ti][0] * lead) <= total * (i + 1) / (NSTEPS + skew):
                    thunks[ti][1]()
                    done += thunks[ti][0]
                    ti += 1
            while ti < len(thunks):
                thunks[ti][1]()
                ti += 1

        def run(thunks):
            for _, th in thunks:
                th()

        cp_x(0).start()
        for j in (1, 0, 2):
            cp_qkv(j).start()
        cp_x(1).start()
        cp_wo.start()
        cp_w1.start()
        cp_w2.start()
        for t in range(2, NB):
            cp_x(t).start()

        a = stage_a(0, first=True)
        with scope("p0ln"):
            run([a["ln"]])
        with scope("p0k"):
            run([a["k"]])
        with scope("p0q"):
            run([a["q"]])
        with scope("p0v"):
            run([a["v"]])

        if nodma:
            for t in range(1, NB):
                cp_x(t).wait()
        if mode == "3stage":
            a = stage_a(1)
            with scope("p1"):
                run_mixed(attention(0), [a["ln"], a["k"], a["v"]])
                cp_wo.wait()
                oproj(0)
                a["q"][1]()
                ln2()
            with scope("p1w"):
                cp_w1.wait()
                cp_w2.wait()

            def body(t, carry):
                if nodma:
                    t = jnp.minimum(t, NB - 2)
                a = stage_a(t + 1)
                fthunks = ffn(t - 1)
                run_mixed(attention(t), [a["ln"]] + fthunks + [a["k"], a["v"]])
                oproj(t)
                a["q"][1]()
                ln2()
                return carry
            with scope("loop"):
                lax.fori_loop(1, NB - 1 + (extra or 0), body, 0)
            with scope("p2"):
                run_mixed(attention(NB - 1), ffn(NB - 2))
                oproj(NB - 1)
                ln2()
                run(ffn(NB - 1))
        elif mode == "3b":
            a = stage_a(1)
            with scope("p1"):
                run_mixed(attention(0), [a["ln"], a["k"], a["v"]])
                cp_wo.wait()
                oproj(0)
                a["q"][1]()
                ln2()
            with scope("p1w"):
                cp_w1.wait()
                cp_w2.wait()

            def body(t, carry):
                if nodma:
                    t = jnp.minimum(t, NB - 2)
                if edge == "start":
                    cp_x(t + 1).wait()
                a = stage_a(t + 1, wait=not edge)
                fthunks = ffn(t - 1, start=not edge)
                for th in fthunks[:pre]:
                    th[1]()
                rest = fthunks[pre:]
                rest.insert(lnpos, a["ln"])
                run_mixed(attention(t), rest)
                for nm in tail:
                    if nm == "o":
                        oproj(t)
                    elif nm == "l":
                        ln2()
                    else:
                        a[nm][1]()
                if edge:
                    for r in range(TQ // FR):
                        cp_out(t - 1, r).start()
                if edge == "end":
                    cp_x(jnp.minimum(t + 2, NB - 1)).wait()
                return carry
            with scope("loop"):
                lax.fori_loop(1, NB - 1 + (extra or 0), body, 0)
            with scope("p2"):
                fthunks = ffn(NB - 2)
                for th in fthunks[:pre]:
                    th[1]()
                run_mixed(attention(NB - 1), fthunks[pre:])
                oproj(NB - 1)
                ln2()
                run(ffn(NB - 1))
        elif mode == "2stage":
            for _ in attention(0):
                pass
            cp_wo.wait()
            cp_w1.wait()
            cp_w2.wait()

            def body(t, carry):
                if nodma:
                    t = jnp.minimum(t, NB - 1)
                a = stage_a(t)
                oproj(t - 1)
                run([a["ln"], a["k"]])
                ln2()
                run([a["q"], a["v"]])
                run_mixed(attention(t), ffn(t - 1))
                return carry
            lax.fori_loop(1, NB + (extra or 0), body, 0)
            oproj(NB - 1)
            ln2()
            run(ffn(NB - 1))
        with scope("fin"):
            for t in range(NB):
                for r in range(TQ // FR):
                    if nodma:
                        cp_out(t, r).start()
                    cp_out(t, r).wait()

    return kernel


def build(LA=4, FR=128, F1C=256, F2C=128, skew=4, PVD=(0, 0), mode="3stage", lead=0.5, extra=None, stS=True, stP=False, pre=0, lnpos=0, tail="kovlq", edge=None):
    @jax.jit
    def fn(A_x, A_wqkv, A_wo, B_x, B_w1, B_w2):
        x = A_x.reshape(S, D)
        anyspec = pl.BlockSpec(memory_space=pl.ANY)
        out = pl.pallas_call(
            make_kernel(LA, FR, F1C, F2C, skew, PVD, mode, lead, extra, stS, stP, pre, lnpos, tail, edge),
            in_specs=[anyspec] * 5,
            out_specs=anyspec,
            out_shape=jax.ShapeDtypeStruct((S, D), BF16),
            scratch_shapes=[pltpu.VMEM((S, D), BF16), pltpu.VMEM((S, D), BF16),
                            pltpu.VMEM((D, 3 * D), BF16), pltpu.VMEM((D, D), BF16),
                            pltpu.VMEM((D, DFF), BF16), pltpu.VMEM((DFF, D), BF16),
                            pltpu.VMEM((D, D), BF16),
                            pltpu.VMEM((NQUAD, S // 2, 128), U32),
                            pltpu.VMEM((S // 128, H * 16, 128), U32),
                            pltpu.VMEM((2, NQUAD, TQ // 2, 128), U32),
                            pltpu.VMEM((TQ, D), BF16), pltpu.VMEM((TQ, D), F32), pltpu.VMEM((TQ, D), BF16),
                            pltpu.VMEM((64, 256, 128), F32), pltpu.VMEM((64, 144, 128), U32),
                            pltpu.SemaphoreType.DMA((6,)), pltpu.SemaphoreType.DMA((NB,)),
                            pltpu.SemaphoreType.DMA((NB * (TQ // FR),))],
            compiler_params=pltpu.CompilerParams(vmem_limit_bytes=100 * 1024 * 1024),
            name="fused",
        )(x, A_wqkv, A_wo, B_w1, B_w2)
        return out.reshape(1, S, D)
    return fn


_FN = build(mode="3b", pre=1, lnpos=10, edge="start")


@jax.jit
def pallas_sequential_preLN__sliding_block__dense_activation_relu__prompt_kernel(A_x, A_wqkv, A_wo, B_x, B_w1, B_w2):
    return _FN(A_x, A_wqkv, A_wo, B_x, B_w1, B_w2)
```

```python
import math

import jax
import jax.numpy as jnp
from jax import lax
from jax.experimental import pallas as pl
from jax.experimental.pallas import tpu as pltpu

S, D, H, DH, W, DFF = 2048, 640, 32, 20, 256, 1536
NQUAD = H // 4
EPS = 1e-5
QSCALE = (DH ** -0.5) * math.log2(math.e)
NEG = -1e30
F32 = jnp.float32
BF16 = jnp.bfloat16
U32 = jnp.uint32
ONES = 0x3F803F80
NT = (((1,), (1,)), ((), ()))
TQ = 256
NSB = TQ // 128
NB = S // TQ
NUNIT = NSB * NQUAD * 4
_ONE_ROW = {0: 20, 4: 0, 8: 28, 12: 8}

MIX_FIRST = (10, 2, 1, 16, 0.5, 0)
MIX_LOOP = (5, 1, 0, 1, 0.5, 1)
MIX_LAST = (6, 2, 0, 4, 0.0, 2)
KA, QA0, QA = 256, 384, 512


def _ln(x):
    mu = jnp.mean(x, axis=-1, keepdims=True)
    xc = x - mu
    var = jnp.mean(xc * xc, axis=-1, keepdims=True)
    return xc * lax.rsqrt(var + EPS)


def _pack(x_bf16):
    return pltpu.bitcast(x_bf16, U32)


def _unpack(x_u32):
    return pltpu.bitcast(x_u32, BF16)


def _ipack(x, rnd=True):
    n, L = x.shape[0] // 16, x.shape[1]
    u = lax.bitcast_convert_type(x, U32)
    if rnd:
        u = u + jnp.uint32(0x8000)
    u3 = u.reshape(n, 16, L)
    lo = u3[:, 0:8, :].reshape(8 * n, L)
    hi = u3[:, 8:16, :].reshape(8 * n, L)
    return lax.shift_right_logical(lo, jnp.uint32(16)) | (hi & jnp.uint32(0xFFFF0000))


def _lane_in(lane, lo, n):
    lo = lo % 128
    hi = lo + n
    if hi <= 128:
        return (lane >= lo) & (lane < hi)
    return (lane >= lo) | (lane < hi - 128)


def _dot(a, b):
    return jnp.dot(a, b, preferred_element_type=F32)


def _rows(t, n):
    return t * n if isinstance(t, int) else pl.multiple_of(t * n, n)


def _kernel(x_hbm, wqkv_hbm, wo_hbm, w1_hbm, w2_hbm, out_hbm,
            x_v, out_v, wqkv_ref, wo_ref, w1_ref, w2_ref, wvt_ref, k_ref, vt_ref, q_ref,
            os_ref, h1_ref, hn_ref, s_ref, isem, osem):

    def cp_wqkv(c0, c1, si):
        cols = pl.ds(c0, c1 - c0)
        return pltpu.make_async_copy(wqkv_hbm.at[:, cols], wqkv_ref.at[:, cols], isem.at[si])

    cp_ka = cp_wqkv(D, D + KA, 0)
    cp_kb = cp_wqkv(D + KA, 2 * D, 1)
    cp_q = cp_wqkv(0, D, 2)
    cp_v = cp_wqkv(2 * D, 3 * D, 3)
    cp_wo = pltpu.make_async_copy(wo_hbm, wo_ref, isem.at[4])
    cp_w1 = pltpu.make_async_copy(w1_hbm, w1_ref, isem.at[5])
    cp_w2 = pltpu.make_async_copy(w2_hbm, w2_ref, isem.at[6])

    def cp_x(t):
        r = pl.ds(_rows(t, TQ), TQ)
        return pltpu.make_async_copy(x_hbm.at[r], x_v.at[r], isem.at[7 + t])

    def cp_out(t, r0=0, nr=TQ, c0=0, c1=D):
        rr = pl.ds(_rows(t, TQ) + r0, nr)
        if c1 - c0 == D:
            return pltpu.make_async_copy(out_v.at[rr], out_hbm.at[rr], osem.at[0])
        cc = pl.ds(c0, c1 - c0)
        return pltpu.make_async_copy(out_v.at[rr, cc], out_hbm.at[rr, cc], osem.at[0])

    last_cps = []

    class StageA:
        def __init__(self, t):
            self.t = t
            self.tiles = {"k": {}, "q": {}}
            self.done = set()
            self.vrows = {}

        def ln(self):
            xnf = _ln(x_v[pl.ds(_rows(self.t, TQ), TQ), :].astype(F32))
            self.xn = xnf.astype(BF16)
            self.xni = _unpack(_ipack(xnf))

        def qk(self, which, c0, c1, rc):
            for r0 in range(0, TQ, rc):
                self.qk_rows(which, c0, c1, r0, rc)

        def qk_rows(self, which, c0, c1, r0, rc):
            t = self.t
            base = D if which == "k" else 0
            y = _dot(self.xn[r0:r0 + rc], wqkv_ref[:, base + c0:base + c1])
            if which == "q":
                y = y * QSCALE
            yp = _pack(y.astype(BF16))
            tiles = self.tiles[which].setdefault(r0, {})
            for j in range(c0 // 128, c1 // 128):
                tiles[j] = yp[:, 128 * j - c0:128 * j - c0 + 128]
            lane = lax.broadcasted_iota(jnp.int32, (rc // 2, 128), 1)
            for m in range(NQUAD):
                t0, t1 = (80 * m) // 128, (80 * m + 79) // 128
                if (which, r0, m) in self.done or t0 not in tiles or t1 not in tiles:
                    continue
                self.done.add((which, r0, m))
                val = tiles[t0] if t0 == t1 else jnp.where(lane >= 64, tiles[t0], tiles[t1])
                if which == "k":
                    k_ref[m, pl.ds(_rows(t, TQ // 2) + r0 // 2, rc // 2), :] = val
                else:
                    q_ref[t % 2, m, r0 // 2:(r0 + rc) // 2, :] = val

        def v(self, c0, c1):
            t = self.t
            vt = lax.dot_general(wvt_ref[c0:c1, :], self.xni, NT, preferred_element_type=F32)
            vtp = _ipack(vt)
            for j in range(c0 // 16, c1 // 16):
                self.vrows[j] = vtp[8 * j - c0 // 2:8 * j - c0 // 2 + 8]
            sub16 = lax.broadcasted_iota(jnp.int32, (16, 128), 0)
            for h in range(H):
                j = (20 * h) // 16
                if ("v", h) in self.done or j not in self.vrows or j + 1 not in self.vrows:
                    continue
                self.done.add(("v", h))
                r1 = _ONE_ROW[20 * h - 16 * j]
                win = jnp.concatenate([self.vrows[j], self.vrows[j + 1]], axis=0)
                for sb in range(NSB):
                    vt_ref[t * NSB + sb, 16 * h:16 * h + 16, :] = jnp.where(
                        sub16 == r1 // 2, jnp.uint32(ONES), win[:, 128 * sb:128 * sb + 128])

    def prep_wvt():
        wp = _pack(wqkv_ref[:, 2 * D:3 * D].T)
        ev = lax.bitcast_convert_type(lax.shift_left(wp, jnp.uint32(16)), F32)
        od = lax.bitcast_convert_type(wp & jnp.uint32(0xFFFF0000), F32)
        wd = jnp.concatenate([ev.reshape(D // 16, 8, D), od.reshape(D // 16, 8, D)], axis=1)
        wvt_ref[...] = wd.reshape(D, D).astype(BF16)

    def attention(t, la):
        clipped = isinstance(t, int) and t == 0
        lane64 = lax.broadcasted_iota(jnp.int32, (64, 128), 1)
        lane16 = lax.broadcasted_iota(jnp.int32, (16, 128), 1)
        tri = (lax.broadcasted_iota(jnp.int32, (32, 128), 0)
               > lax.broadcasted_iota(jnp.int32, (32, 128), 1) % 32)
        row16 = lax.broadcasted_iota(jnp.int32, (16, 128), 0)
        row_lo = row16 + (row16 & 8)
        trip = (jnp.where(row_lo > lane16 % 32, jnp.uint32(0xFFFF), jnp.uint32(0))
                | jnp.where(row_lo + 8 > lane16 % 32, jnp.uint32(0xFFFF0000), jnp.uint32(0)))
        sub8 = lax.broadcasted_iota(jnp.int32, (8, 128), 0)
        odd = (lane16 & 32) != 0
        hi = (lane16 & 64) != 0

        def sel(msk, tv, fv):
            if tv is None and fv is None:
                return None
            z = jnp.zeros((16, 128), U32)
            return jnp.where(msk, z if tv is None else tv, z if fv is None else fv)

        def stage_q(sb, m):
            qt = q_ref[t % 2, m, 64 * sb:64 * sb + 64, :]
            return [jnp.where(_lane_in(lane64, 80 * m + 20 * k, 20), qt, jnp.uint32(0)) for k in range(4)]

        def stage_s(sb, m, g, qm):
            rhs = _unpack(jnp.concatenate([qm[(g - p) % 4][16 * g:16 * g + 16] for p in range(4)], axis=0))
            if clipped:
                n = 128 * sb + 32 * (g + 1)
                s = lax.dot_general(_unpack(k_ref[m, 0:n // 2, :]), rhs, NT, preferred_element_type=F32)
                last = jnp.where(tri, NEG, s[n - 32:n])
                mm = jnp.concatenate([s[0:n - 32], last], axis=0) if n > 32 else last
            else:
                r0 = (t * NSB + sb - 2) * 64 + 16 * g
                if not isinstance(r0, int):
                    r0 = pl.multiple_of(r0, 16)
                s = lax.dot_general(_unpack(k_ref[m, pl.ds(r0, 144), :]), rhs, NT, preferred_element_type=F32)
                mm = jnp.concatenate([jnp.where(tri, s[0:32], s[256:288]), s[32:256]], axis=0)
            return mm, jnp.max(mm, axis=0, keepdims=True)

        def stage_e(mm, mx):
            p = _ipack(jnp.exp2(mm - mx), False)
            if clipped:
                return p
            return jnp.concatenate([p[0:16] & trip, p[16:128], p[0:16] & ~trip], axis=0)

        def stage_pv(sb, m, P, par):
            if clipped:
                nR, off, vb0 = 4 * (sb + 1), [0, 0, 0, 0], 0
            else:
                nR, off, vb0 = 12, [0, 1, 2, 3], t * NSB + sb - 2
            blocks = {par: [], par + 2: []}
            for R in range(nR):
                A = []
                for g in range(4):
                    j = R - off[g]
                    A.append(P[g][16 * j:16 * j + 16] if 0 <= j < P[g].shape[0] // 16 else None)
                b0 = sel(odd, A[(par + 1) % 4], A[par])
                b2 = sel(odd, A[(par + 3) % 4], A[par + 2])
                for k, o in ((par, sel(hi, b2, b0)), (par + 2, sel(hi, b0, b2))):
                    blocks[k].append(jnp.zeros((16, 128), U32) if o is None else o)
            res = {}
            for k in (par, par + 2):
                h = 4 * m + k
                ws = 16 * ((20 * h) // 16)
                r1 = _ONE_ROW[20 * h - ws]
                pk = _unpack(jnp.concatenate(blocks[k], axis=0))
                vws = [vt_ref[vb0 + i, 16 * h:16 * h + 16, :] for i in range(nR // 4)]
                vwin = jnp.concatenate(vws, axis=1) if len(vws) > 1 else vws[0]
                o = _dot(_unpack(vwin), pk)
                a = 8 * ((20 * h) // 8) - ws
                o = o[a:a + 24] * (1.0 / o[r1:r1 + 1])
                res[k] = pltpu.roll(o, 32 * k, 1) if k else o
            return res

        units = [(sb, m, g) for sb in range(NSB) for m in range(NQUAD) for g in range(4)]
        Sv, Pv, rows = {}, {}, []
        qm = None
        for u in range(-la, NUNIT):
            us = u + la
            if us < NUNIT:
                sb, m, g = units[us]
                if g == 0:
                    qm = stage_q(sb, m)
                mm, mx = stage_s(sb, m, g, qm)
                s_ref[us, 0:mm.shape[0], :] = mm
                Sv[us] = (mm.shape[0], mx)
            if u >= 0:
                nr, mx = Sv.pop(u)
                Pv[u] = stage_e(s_ref[u, 0:nr, :], mx)
                sb, m, g = units[u]
                if g == 3:
                    P = [Pv.pop(u - 3 + i) for i in range(4)]
                    o24 = stage_pv(sb, m, P, 0)
                    o24.update(stage_pv(sb, m, P, 1))
                    for pr in range(2):
                        ev, od = o24[2 * pr], o24[2 * pr + 1]
                        rows += [ev[0:16], jnp.where(sub8 < 4, ev[16:24], od[0:8]), od[8:24]]
                    if m == NQUAD - 1:
                        ot = jnp.concatenate(rows, axis=0)
                        rows = []
                        os_ref[128 * sb:128 * sb + 128, :] = ot.T.astype(BF16)
            yield

    def oproj(t, rc):
        for r0 in range(0, TQ, rc):
            h1_ref[r0:r0 + rc, :] = (x_v[pl.ds(_rows(t, TQ) + r0, rc), :].astype(F32)
                                     + _dot(os_ref[r0:r0 + rc, :], wo_ref[...]))

    def ln2():
        hn_ref[...] = _ln(h1_ref[...]).astype(BF16)

    def ffn(t, frc, f1c, f2c, start=False):
        thunks = []
        f = {}
        for r in range(TQ // frc):
            rs = slice(frc * r, frc * r + frc)
            for j in range(DFF // f1c):
                def t1(r=r, rs=rs, j=j):
                    f[(r, j)] = jnp.maximum(
                        _dot(hn_ref[rs, :], w1_ref[:, f1c * j:f1c * j + f1c]), 0.0).astype(BF16)
                thunks.append((frc * 5 * (f1c // 128), t1))
            for c0 in range(0, D, f2c):
                c1 = min(D, c0 + f2c)

                def t2(r=r, rs=rs, c0=c0, c1=c1):
                    acc = h1_ref[rs, c0:c1]
                    for j in range(DFF // f1c):
                        acc = acc + _dot(f[(r, j)], w2_ref[f1c * j:f1c * j + f1c, c0:c1])
                    out_v[pl.ds(_rows(t, TQ) + frc * r, frc), c0:c1] = acc.astype(BF16)
                    if start and (r == TQ // frc - 1 or c1 == D):
                        if r == TQ // frc - 1:
                            last_cps.append(cp_out(t, frc * r, frc, c0, c1))
                        else:
                            last_cps.append(cp_out(t, frc * r, frc))
                        last_cps[-1].start()
                thunks.append((frc * 12 * ((c1 - c0) // 128), t2))
        return thunks

    def run_mixed(t, thunks, mix):
        la, gr, go, skew, lead, pre = mix
        for _, th in thunks[:pre]:
            th()
        thunks = thunks[pre:]
        total = sum(w for w, _ in thunks)
        done, ti = 0, 0
        for i, _ in enumerate(attention(t, la)):
            while (i % gr == go and ti < len(thunks)
                   and done + thunks[ti][0] * lead <= total * (i + 1) / (NUNIT + la + skew)):
                thunks[ti][1]()
                done += thunks[ti][0]
                ti += 1
        for _, th in thunks[ti:]:
            th()

    for cp in ([cp_x(0), cp_x(1), cp_ka, cp_kb, cp_q, cp_v, cp_wo, cp_w1, cp_w2]
               + [cp_x(t) for t in range(2, NB)]):
        cp.start()

    a0, a1 = StageA(0), StageA(1)
    cp_x(0).wait()
    a0.ln()
    cp_x(1).wait()
    a1.ln()
    cp_ka.wait()
    a0.qk("k", 0, KA, 128)
    a1.qk("k", 0, KA, 128)
    cp_kb.wait()
    a0.qk("k", KA, D, 128)
    a1.qk("k", KA, D, 128)
    cp_q.wait()
    a0.qk("q", 0, D, 128)
    a1.qk("q", 0, QA0, 128)
    cp_v.wait()
    cp_wo.wait()
    prep_wvt()
    a1.qk("q", QA0, QA, 128)
    a0.v(0, D)
    run_mixed(0, [(1, lambda: a1.v(0, D // 2)), (1, lambda: a1.v(D // 2, D))], MIX_FIRST)
    oproj(0, 128)
    a1.qk("q", QA, D, 128)
    ln2()
    cp_w1.wait()
    cp_w2.wait()

    def body(t, carry):
        cp_x(t + 1).wait()
        a = StageA(t + 1)
        a.ln()
        run_mixed(t, ffn(t - 1, 64, 256, 128), MIX_LOOP)
        a.qk("k", 0, D, 64)
        oproj(t, 128)
        ln2()
        for c0 in range(0, D, 128):
            a.v(c0, c0 + 128)
        a.qk("q", 0, D, 64)
        cp_out(t - 1).start()
        return carry

    lax.fori_loop(1, NB - 1, body, 0)

    run_mixed(NB - 1, ffn(NB - 2, 64, 256, 128), MIX_LAST)
    cp_out(NB - 2).start()
    oproj(NB - 1, 64)
    ln2()
    for _, th in ffn(NB - 1, 64, 512, 256, start=True):
        th()
    for t in range(NB - 1):
        cp_out(t).wait()
    for cp in last_cps:
        cp.wait()


@jax.jit
def pallas_sequential_preLN__sliding_block__dense_activation_relu__prompt_kernel(
        A_x: jax.Array,
        A_wqkv: jax.Array,
        A_wo: jax.Array,
        B_x: jax.Array,
        B_w1: jax.Array,
        B_w2: jax.Array,
):
    anyspec = pl.BlockSpec(memory_space=pl.ANY)
    out = pl.pallas_call(
        _kernel,
        in_specs=[anyspec] * 5,
        out_specs=anyspec,
        out_shape=jax.ShapeDtypeStruct((S, D), BF16),
        scratch_shapes=[
            pltpu.VMEM((S, D), BF16), pltpu.VMEM((S, D), BF16),
            pltpu.VMEM((D, 3 * D), BF16), pltpu.VMEM((D, D), BF16),
            pltpu.VMEM((D, DFF), BF16), pltpu.VMEM((DFF, D), BF16),
            pltpu.VMEM((D, D), BF16),
            pltpu.VMEM((NQUAD, S // 2, 128), U32),
            pltpu.VMEM((S // 128, H * 16, 128), U32),
            pltpu.VMEM((2, NQUAD, TQ // 2, 128), U32),
            pltpu.VMEM((TQ, D), BF16),
            pltpu.VMEM((TQ, D), F32), pltpu.VMEM((TQ, D), BF16),
            pltpu.VMEM((NUNIT, 256, 128), F32),
            pltpu.SemaphoreType.DMA((7 + NB,)), pltpu.SemaphoreType.DMA((1,))],
        compiler_params=pltpu.CompilerParams(
            vmem_limit_bytes=100 * 1024 * 1024,
            disable_bounds_checks=True, disable_semaphore_checks=True),
        name="fused",
    )(A_x.reshape(S, D), A_wqkv, A_wo, B_w1, B_w2)
    return out.reshape(1, S, D)
```

```python
import math

import jax
import jax.numpy as jnp
from jax import lax
from jax.experimental import pallas as pl
from jax.experimental.pallas import tpu as pltpu

S, D, H, DH, W, DFF = 2048, 640, 32, 20, 256, 1536
NQUAD = H // 4
EPS = 1e-5
QSCALE = (DH ** -0.5) * math.log2(math.e)
NEG = -1e30
F32 = jnp.float32
BF16 = jnp.bfloat16
U32 = jnp.uint32
ONES = 0x3F803F80
NT = (((1,), (1,)), ((), ()))
TQ = 256
NSB = TQ // 128
NB = S // TQ
NUNIT = NSB * NQUAD * 4
_ONE_ROW = {0: 20, 4: 0, 8: 28, 12: 8}

MIX_FIRST = (10, (
    18, 68,
))
MIX_LOOP = (5, (
    -1, -1, 2, 3, 5, 6, 8, 8, 11, 13, 15, 17, 18, 20, 21, 23, 24, 25, 26, 29, 31, 33, 34, 36,
    36, 39, 40, 42, 44, 45, 47, 49, 51, 52, 54, 55, 57, 57, 61, 62, 64, 65, 67, 99,
))
MIX_LAST = (6, (
    -1, -1, 0, 2, 4, 4, 6, 8, 10, 12, 14, 17, 18, 20, 21, 21, 24, 26, 28, 30, 32, 34, 36, 36,
    38, 42, 42, 46, 46, 46, 48, 50, 52, 54, 56, 58, 60, 62, 63, 64, 66, 68, 72, 99,
))
KA, QA0, QA = 256, 384, 512


def _ln(x):
    mu = jnp.mean(x, axis=-1, keepdims=True)
    xc = x - mu
    var = jnp.mean(xc * xc, axis=-1, keepdims=True)
    return xc * lax.rsqrt(var + EPS)


def _pack(x_bf16):
    return pltpu.bitcast(x_bf16, U32)


def _unpack(x_u32):
    return pltpu.bitcast(x_u32, BF16)


def _ipack(x, rnd=True):
    n, L = x.shape[0] // 16, x.shape[1]
    u = lax.bitcast_convert_type(x, U32)
    if rnd:
        u = u + jnp.uint32(0x8000)
    u3 = u.reshape(n, 16, L)
    lo = u3[:, 0:8, :].reshape(8 * n, L)
    hi = u3[:, 8:16, :].reshape(8 * n, L)
    return lax.shift_right_logical(lo, jnp.uint32(16)) | (hi & jnp.uint32(0xFFFF0000))


def _lane_in(lane, lo, n):
    lo = lo % 128
    hi = lo + n
    if hi <= 128:
        return (lane >= lo) & (lane < hi)
    return (lane >= lo) | (lane < hi - 128)


def _dot(a, b):
    return jnp.dot(a, b, preferred_element_type=F32)


def _rows(t, n):
    return t * n if isinstance(t, int) else pl.multiple_of(t * n, n)


def _kernel(x_hbm, wqkv_hbm, wo_hbm, w1_hbm, w2_hbm, out_hbm,
            x_v, out_v, wqkv_ref, wo_ref, w1_ref, w2_ref, wvt_ref, k_ref, vt_ref, q_ref,
            os_ref, h1_ref, hn_ref, s_ref, isem, osem):

    def cp_wqkv(c0, c1, si):
        cols = pl.ds(c0, c1 - c0)
        return pltpu.make_async_copy(wqkv_hbm.at[:, cols], wqkv_ref.at[:, cols], isem.at[si])

    cp_ka = cp_wqkv(D, D + KA, 0)
    cp_kb = cp_wqkv(D + KA, 2 * D, 1)
    cp_q = cp_wqkv(0, D, 2)
    cp_v = cp_wqkv(2 * D, 3 * D, 3)
    cp_wo = pltpu.make_async_copy(wo_hbm, wo_ref, isem.at[4])
    cp_w1 = pltpu.make_async_copy(w1_hbm, w1_ref, isem.at[5])
    cp_w2 = pltpu.make_async_copy(w2_hbm, w2_ref, isem.at[6])

    def cp_x(t):
        r = pl.ds(_rows(t, TQ), TQ)
        return pltpu.make_async_copy(x_hbm.at[r], x_v.at[r], isem.at[7 + t])

    def cp_out(t, r0=0, nr=TQ, c0=0, c1=D):
        rr = pl.ds(_rows(t, TQ) + r0, nr)
        if c1 - c0 == D:
            return pltpu.make_async_copy(out_v.at[rr], out_hbm.at[rr], osem.at[0])
        cc = pl.ds(c0, c1 - c0)
        return pltpu.make_async_copy(out_v.at[rr, cc], out_hbm.at[rr, cc], osem.at[0])

    last_cps = []

    class StageA:
        def __init__(self, t):
            self.t = t
            self.tiles = {"k": {}, "q": {}}
            self.done = set()
            self.vrows = {}

        def ln(self):
            xnf = _ln(x_v[pl.ds(_rows(self.t, TQ), TQ), :].astype(F32))
            self.xn = xnf.astype(BF16)
            self.xni = _unpack(_ipack(xnf))

        def qk(self, which, c0, c1, rc):
            for r0 in range(0, TQ, rc):
                self.qk_rows(which, c0, c1, r0, rc)

        def qk_rows(self, which, c0, c1, r0, rc):
            t = self.t
            base = D if which == "k" else 0
            y = _dot(self.xn[r0:r0 + rc], wqkv_ref[:, base + c0:base + c1])
            if which == "q":
                y = y * QSCALE
            yp = _pack(y.astype(BF16))
            tiles = self.tiles[which].setdefault(r0, {})
            for j in range(c0 // 128, c1 // 128):
                tiles[j] = yp[:, 128 * j - c0:128 * j - c0 + 128]
            lane = lax.broadcasted_iota(jnp.int32, (rc // 2, 128), 1)
            for m in range(NQUAD):
                t0, t1 = (80 * m) // 128, (80 * m + 79) // 128
                if (which, r0, m) in self.done or t0 not in tiles or t1 not in tiles:
                    continue
                self.done.add((which, r0, m))
                val = tiles[t0] if t0 == t1 else jnp.where(lane >= 64, tiles[t0], tiles[t1])
                if which == "k":
                    k_ref[m, pl.ds(_rows(t, TQ // 2) + r0 // 2, rc // 2), :] = val
                else:
                    q_ref[t % 2, m, r0 // 2:(r0 + rc) // 2, :] = val

        def v(self, c0, c1):
            t = self.t
            vt = lax.dot_general(wvt_ref[c0:c1, :], self.xni, NT, preferred_element_type=F32)
            vtp = _ipack(vt)
            for j in range(c0 // 16, c1 // 16):
                self.vrows[j] = vtp[8 * j - c0 // 2:8 * j - c0 // 2 + 8]
            sub16 = lax.broadcasted_iota(jnp.int32, (16, 128), 0)
            for h in range(H):
                j = (20 * h) // 16
                if ("v", h) in self.done or j not in self.vrows or j + 1 not in self.vrows:
                    continue
                self.done.add(("v", h))
                r1 = _ONE_ROW[20 * h - 16 * j]
                win = jnp.concatenate([self.vrows[j], self.vrows[j + 1]], axis=0)
                for sb in range(NSB):
                    vt_ref[t * NSB + sb, 16 * h:16 * h + 16, :] = jnp.where(
                        sub16 == r1 // 2, jnp.uint32(ONES), win[:, 128 * sb:128 * sb + 128])

    def prep_wvt():
        wp = _pack(wqkv_ref[:, 2 * D:3 * D].T)
        ev = lax.bitcast_convert_type(lax.shift_left(wp, jnp.uint32(16)), F32)
        od = lax.bitcast_convert_type(wp & jnp.uint32(0xFFFF0000), F32)
        wd = jnp.concatenate([ev.reshape(D // 16, 8, D), od.reshape(D // 16, 8, D)], axis=1)
        wvt_ref[...] = wd.reshape(D, D).astype(BF16)

    def attention(t, la):
        clipped = isinstance(t, int) and t == 0
        lane64 = lax.broadcasted_iota(jnp.int32, (64, 128), 1)
        lane16 = lax.broadcasted_iota(jnp.int32, (16, 128), 1)
        tri = (lax.broadcasted_iota(jnp.int32, (32, 128), 0)
               > lax.broadcasted_iota(jnp.int32, (32, 128), 1) % 32)
        row16 = lax.broadcasted_iota(jnp.int32, (16, 128), 0)
        row_lo = row16 + (row16 & 8)
        trip = (jnp.where(row_lo > lane16 % 32, jnp.uint32(0xFFFF), jnp.uint32(0))
                | jnp.where(row_lo + 8 > lane16 % 32, jnp.uint32(0xFFFF0000), jnp.uint32(0)))
        sub8 = lax.broadcasted_iota(jnp.int32, (8, 128), 0)
        odd = (lane16 & 32) != 0
        hi = (lane16 & 64) != 0

        def sel(msk, tv, fv):
            if tv is None and fv is None:
                return None
            z = jnp.zeros((16, 128), U32)
            return jnp.where(msk, z if tv is None else tv, z if fv is None else fv)

        def stage_q(sb, m):
            qt = q_ref[t % 2, m, 64 * sb:64 * sb + 64, :]
            return [jnp.where(_lane_in(lane64, 80 * m + 20 * k, 20), qt, jnp.uint32(0)) for k in range(4)]

        def stage_s(sb, m, g, qm):
            rhs = _unpack(jnp.concatenate([qm[(g - p) % 4][16 * g:16 * g + 16] for p in range(4)], axis=0))
            if clipped:
                n = 128 * sb + 32 * (g + 1)
                s = lax.dot_general(_unpack(k_ref[m, 0:n // 2, :]), rhs, NT, preferred_element_type=F32)
                last = jnp.where(tri, NEG, s[n - 32:n])
                mm = jnp.concatenate([s[0:n - 32], last], axis=0) if n > 32 else last
            else:
                r0 = (t * NSB + sb - 2) * 64 + 16 * g
                if not isinstance(r0, int):
                    r0 = pl.multiple_of(r0, 16)
                s = lax.dot_general(_unpack(k_ref[m, pl.ds(r0, 144), :]), rhs, NT, preferred_element_type=F32)
                mm = jnp.concatenate([jnp.where(tri, s[0:32], s[256:288]), s[32:256]], axis=0)
            return mm, jnp.max(mm, axis=0, keepdims=True)

        def stage_e(mm, mx):
            p = _ipack(jnp.exp2(mm - mx), False)
            if clipped:
                return p
            return jnp.concatenate([p[0:16] & trip, p[16:128], p[0:16] & ~trip], axis=0)

        def stage_pv(sb, m, P, par):
            if clipped:
                nR, off, vb0 = 4 * (sb + 1), [0, 0, 0, 0], 0
            else:
                nR, off, vb0 = 12, [0, 1, 2, 3], t * NSB + sb - 2
            blocks = {par: [], par + 2: []}
            for R in range(nR):
                A = []
                for g in range(4):
                    j = R - off[g]
                    A.append(P[g][16 * j:16 * j + 16] if 0 <= j < P[g].shape[0] // 16 else None)
                b0 = sel(odd, A[(par + 1) % 4], A[par])
                b2 = sel(odd, A[(par + 3) % 4], A[par + 2])
                for k, o in ((par, sel(hi, b2, b0)), (par + 2, sel(hi, b0, b2))):
                    blocks[k].append(jnp.zeros((16, 128), U32) if o is None else o)
            res = {}
            for k in (par, par + 2):
                h = 4 * m + k
                ws = 16 * ((20 * h) // 16)
                r1 = _ONE_ROW[20 * h - ws]
                pk = _unpack(jnp.concatenate(blocks[k], axis=0))
                vws = [vt_ref[vb0 + i, 16 * h:16 * h + 16, :] for i in range(nR // 4)]
                vwin = jnp.concatenate(vws, axis=1) if len(vws) > 1 else vws[0]
                o = _dot(_unpack(vwin), pk)
                a = 8 * ((20 * h) // 8) - ws
                o = o[a:a + 24] * (1.0 / o[r1:r1 + 1])
                res[k] = pltpu.roll(o, 32 * k, 1) if k else o
            return res

        units = [(sb, m, g) for sb in range(NSB) for m in range(NQUAD) for g in range(4)]
        Sv, Pv, rows = {}, {}, []
        qm = None
        for u in range(-la, NUNIT):
            us = u + la
            if us < NUNIT:
                sb, m, g = units[us]
                if g == 0:
                    qm = stage_q(sb, m)
                mm, mx = stage_s(sb, m, g, qm)
                s_ref[us, 0:mm.shape[0], :] = mm
                Sv[us] = (mm.shape[0], mx)
            if u >= 0:
                nr, mx = Sv.pop(u)
                Pv[u] = stage_e(s_ref[u, 0:nr, :], mx)
                sb, m, g = units[u]
                if g == 3:
                    P = [Pv.pop(u - 3 + i) for i in range(4)]
                    o24 = stage_pv(sb, m, P, 0)
                    o24.update(stage_pv(sb, m, P, 1))
                    for pr in range(2):
                        ev, od = o24[2 * pr], o24[2 * pr + 1]
                        rows += [ev[0:16], jnp.where(sub8 < 4, ev[16:24], od[0:8]), od[8:24]]
                    if m == NQUAD - 1:
                        ot = jnp.concatenate(rows, axis=0)
                        rows = []
                        os_ref[128 * sb:128 * sb + 128, :] = ot.T.astype(BF16)
            yield

    def oproj(t, rc):
        for r0 in range(0, TQ, rc):
            h1_ref[r0:r0 + rc, :] = (x_v[pl.ds(_rows(t, TQ) + r0, rc), :].astype(F32)
                                     + _dot(os_ref[r0:r0 + rc, :], wo_ref[...]))

    def ln2():
        hn_ref[...] = _ln(h1_ref[...]).astype(BF16)

    def ffn(t, frc, f1c, f2c, start=False):
        thunks = []
        f = {}
        for r in range(TQ // frc):
            rs = slice(frc * r, frc * r + frc)
            for j in range(DFF // f1c):
                def t1(r=r, rs=rs, j=j):
                    f[(r, j)] = jnp.maximum(
                        _dot(hn_ref[rs, :], w1_ref[:, f1c * j:f1c * j + f1c]), 0.0).astype(BF16)
                thunks.append(t1)
            for c0 in range(0, D, f2c):
                c1 = min(D, c0 + f2c)

                def t2(r=r, rs=rs, c0=c0, c1=c1):
                    acc = h1_ref[rs, c0:c1]
                    for j in range(DFF // f1c):
                        acc = acc + _dot(f[(r, j)], w2_ref[f1c * j:f1c * j + f1c, c0:c1])
                    out_v[pl.ds(_rows(t, TQ) + frc * r, frc), c0:c1] = acc.astype(BF16)
                    if start and (r == TQ // frc - 1 or c1 == D):
                        if r == TQ // frc - 1:
                            last_cps.append(cp_out(t, frc * r, frc, c0, c1))
                        else:
                            last_cps.append(cp_out(t, frc * r, frc))
                        last_cps[-1].start()
                thunks.append(t2)
        return thunks

    def run_mixed(t, thunks, mix):
        la, pos = mix
        ti = 0
        while ti < len(thunks) and pos[ti] < 0:
            thunks[ti]()
            ti += 1
        for i, _ in enumerate(attention(t, la)):
            while ti < len(thunks) and pos[ti] <= i:
                thunks[ti]()
                ti += 1
        for th in thunks[ti:]:
            th()

    for cp in ([cp_x(0), cp_x(1), cp_ka, cp_kb, cp_q, cp_v, cp_wo, cp_w1, cp_w2]
               + [cp_x(t) for t in range(2, NB)]):
        cp.start()

    a0, a1 = StageA(0), StageA(1)
    cp_x(0).wait()
    a0.ln()
    cp_x(1).wait()
    a1.ln()
    cp_ka.wait()
    a0.qk("k", 0, KA, 128)
    a1.qk("k", 0, KA, 128)
    cp_kb.wait()
    a0.qk("k", KA, D, 128)
    a1.qk("k", KA, D, 128)
    cp_q.wait()
    a0.qk("q", 0, D, 128)
    a1.qk("q", 0, QA0, 128)
    cp_v.wait()
    cp_wo.wait()
    prep_wvt()
    a1.qk("q", QA0, QA, 128)
    a0.v(0, D)
    run_mixed(0, [lambda: a1.v(0, D // 2), lambda: a1.v(D // 2, D)], MIX_FIRST)
    oproj(0, 128)
    a1.qk("q", QA, D, 128)
    ln2()
    cp_w1.wait()
    cp_w2.wait()

    def body(t, carry):
        cp_x(t + 1).wait()
        a = StageA(t + 1)
        a.ln()
        run_mixed(t, ffn(t - 1, 64, 256, 128), MIX_LOOP)
        a.qk("k", 0, D, 64)
        oproj(t, 128)
        ln2()
        for c0 in range(0, D, 128):
            a.v(c0, c0 + 128)
        a.qk("q", 0, D, 64)
        cp_out(t - 1).start()
        return carry

    lax.fori_loop(1, NB - 1, body, 0)

    run_mixed(NB - 1, ffn(NB - 2, 64, 256, 128), MIX_LAST)
    cp_out(NB - 2).start()
    oproj(NB - 1, 64)
    ln2()
    for th in ffn(NB - 1, 64, 512, 256, start=True):
        th()
    for t in range(NB - 1):
        cp_out(t).wait()
    for cp in last_cps:
        cp.wait()


@jax.jit
def pallas_sequential_preLN__sliding_block__dense_activation_relu__prompt_kernel(
        A_x: jax.Array,
        A_wqkv: jax.Array,
        A_wo: jax.Array,
        B_x: jax.Array,
        B_w1: jax.Array,
        B_w2: jax.Array,
):
    anyspec = pl.BlockSpec(memory_space=pl.ANY)
    out = pl.pallas_call(
        _kernel,
        in_specs=[anyspec] * 5,
        out_specs=anyspec,
        out_shape=jax.ShapeDtypeStruct((S, D), BF16),
        scratch_shapes=[
            pltpu.VMEM((S, D), BF16), pltpu.VMEM((S, D), BF16),
            pltpu.VMEM((D, 3 * D), BF16), pltpu.VMEM((D, D), BF16),
            pltpu.VMEM((D, DFF), BF16), pltpu.VMEM((DFF, D), BF16),
            pltpu.VMEM((D, D), BF16),
            pltpu.VMEM((NQUAD, S // 2, 128), U32),
            pltpu.VMEM((S // 128, H * 16, 128), U32),
            pltpu.VMEM((2, NQUAD, TQ // 2, 128), U32),
            pltpu.VMEM((TQ, D), BF16),
            pltpu.VMEM((TQ, D), F32), pltpu.VMEM((TQ, D), BF16),
            pltpu.VMEM((NUNIT, 256, 128), F32),
            pltpu.SemaphoreType.DMA((7 + NB,)), pltpu.SemaphoreType.DMA((1,))],
        compiler_params=pltpu.CompilerParams(
            vmem_limit_bytes=100 * 1024 * 1024,
            disable_bounds_checks=True, disable_semaphore_checks=True),
        name="fused",
    )(A_x.reshape(S, D), A_wqkv, A_wo, B_w1, B_w2)
    return out.reshape(1, S, D)
```
